```python
import jax
import jax.numpy as jnp

def _softmax(x, axis=-1):
    return jax.nn.softmax(x, axis=axis)
def _gelu(x):
    return jax.nn.gelu(x, approximate=True)
def _silu(x):
    return jax.nn.silu(x)
def _sigmoid(x):
    return jax.nn.sigmoid(x)
def _layernorm(x, axis=-1, eps=1e-5):
    m = jnp.mean(x, axis=axis, keepdims=True)
    v = jnp.var(x, axis=axis, keepdims=True)
    return (x - m) / jnp.sqrt(v + eps)
def _scatter_add(tgt, idx, src, axis=0):
    return tgt.at[idx].add(src)
def _segment_sum(src, seg, n):
    return jax.ops.segment_sum(src, seg, n)
class _Rng:
    def __init__(self, key):
        self._k = key
    def _next(self):
        self._k, sub = jax.random.split(self._k)
        return sub
    def normal(self, shape):
        return jax.random.normal(self._next(), shape, dtype=jnp.bfloat16)
    def randint(self, lo, hi, shape):
        return jax.random.randint(self._next(), shape, lo, hi, dtype=jnp.int32)
    def uniform(self, shape, lo=0.0, hi=1.0):
        return jax.random.uniform(self._next(), shape, jnp.bfloat16, lo, hi)
    def permutation(self, n):
        return jax.random.permutation(self._next(), n)


kernel_name = 'standalone__sliding_block_cached__decode'

def _fwd_setup_inputs():
    _rng = _Rng(jax.random.key(int.from_bytes(__import__("os").urandom(4), "little")))
    _w = (lambda a: (lambda t: t.astype(jnp.bfloat16) if jnp.issubdtype(t.dtype, jnp.floating) else t)(jnp.asarray(a)))
    B, Sq, D = 2, 1, 640
    Hq, Hkv, Sk, Dh = 32, 32, 4096, 128
    assert Hq % Hkv == 0, (Hq, Hkv)
    return {
        "x": _w((lambda *s: _rng.normal(s) * 0.05)(B, Sq, D)),
        "k_cache": _w((lambda *s: _rng.normal(s) * 0.05)(B, Hkv, Sk, Dh)),
        "v_cache": _w((lambda *s: _rng.normal(s) * 0.05)(B, Hkv, Sk, Dh)),
        "wq": _w((lambda *s: _rng.normal(s) * 0.05)(D, Hq * Dh) * (D ** -0.5)),
        "wo": _w((lambda *s: _rng.normal(s) * 0.05)(Hq * Dh, D) * ((Hq * Dh) ** -0.5)),
    }

def _fwd_reference(x, k_cache, v_cache, wq, wo):
    B, Sq, D = x.shape
    Hq, Dh = 32, 128
    Hkv, Sk = k_cache.shape[1], k_cache.shape[2]
    W = min(4096, max(256, Sk // 4))
    rep = Hq // Hkv
    q = (lambda x, *d: x.transpose(*d))((x @ wq).reshape(B, Sq, Hq, Dh), 0, 2, 1, 3)
    k = jnp.repeat(k_cache[:, :, Sk - W:, :], rep, axis=1)
    v = jnp.repeat(v_cache[:, :, Sk - W:, :], rep, axis=1)
    scores = jnp.einsum("bhqd,bhkd->bhqk", q, k) * (Dh ** -0.5)
    p = _softmax(scores, axis=-1)
    o = jnp.einsum("bhqk,bhkd->bhqd", p, v)
    return (lambda x, *d: x.transpose(*d))(o, 0, 2, 1, 3).reshape(B, Sq, Hq * Dh) @ wo


def setup_inputs():
    _inp = _fwd_setup_inputs()
    _gk = jax.random.fold_in(jax.random.key(int.from_bytes(__import__("os").urandom(4), "little")), 2**31 - 1)
    _shapes = [[2, 1, 640]]
    _dtypes = ['bfloat16']
    _gks = jax.random.split(_gk, len(_shapes))
    _gs = [jax.random.normal(k, s, dtype=jnp.dtype(d)) * 0.05 for k, s, d in zip(_gks, _shapes, _dtypes)]
    _inp["grad_out"] = _gs[0]
    return _inp

def reference(x, k_cache, v_cache, wq, wo, grad_out):
    _const = dict()
    def _f(*_d):
        return _fwd_reference(**{'x': _d[0], 'k_cache': _d[1], 'v_cache': _d[2], 'wq': _d[3], 'wo': _d[4], **_const})
    _out, _vjp = jax.vjp(_f, x, k_cache, v_cache, wq, wo)
    _grads = _vjp(grad_out)
    _out0 = jnp.asarray(_out)
    return (_out0, *[jnp.asarray(_g) for _g in _grads])
```

```python
import functools
import jax
import jax.numpy as jnp
import jax.experimental.pallas as pl
import jax.experimental.pallas.tpu as pltpu

F32 = jnp.float32
BF16 = jnp.bfloat16


def build(ZS=16, ZR=128, DEPTH=12, PER_STEP=6, RG=8, LAST_EARLY=1, do_compute=True, do_writes=True,
          WQ_S=10, WQ_R=8, WO_S=8, WO_R=32):
    def fn(x, k_cache, v_cache, wq, wo, grad_out):
        B, Sq, D = x.shape
        _, H, Sk, Dh = k_cache.shape
        W = min(4096, max(256, Sk // 4))
        Z = Sk - W
        BH = B * H
        scale = Dh ** -0.5
        HD = H * Dh
        nG = BH // RG
        nzs = BH // ZS
        nzr = Z // ZR
        ndr = W // ZR
        n_zero = 2 * nzs * nzr
        n_data = 2 * nzs * ndr
        wq_rows = D // WQ_S
        wo_rows = HD // WO_S
        n_wq = wq_rows // WQ_R
        n_wo = wo_rows // WO_R

        def kernel(x_hbm, k_hbm, v_hbm, wq_hbm, wo_hbm, go_hbm,
                   out_hbm, dx_hbm, dk_hbm, dv_hbm, dwq_hbm, dwo_hbm,
                   x_v, go_v, out_v, dx_v, wq_v, wo_v, k_v, v_v, dk_v, dv_v, dwq_v, dwo_v,
                   zbuf, q_s, do_s, acc_out, acc_dx,
                   rsem, ksem, vsem, wsem, osem):
            c_x = pltpu.make_async_copy(x_hbm, x_v, rsem.at[0])
            c_go = pltpu.make_async_copy(go_hbm, go_v, rsem.at[1])
            c_wq = pltpu.make_async_copy(wq_hbm, wq_v, rsem.at[2])
            c_wo = pltpu.make_async_copy(wo_hbm, wo_v, rsem.at[3])
            c_wq.start(); c_x.start(); c_go.start(); c_wo.start()

            def kcp(g):
                return pltpu.make_async_copy(k_hbm.at[pl.ds(g * RG, RG), pl.ds(Z, W)],
                                             k_v.at[pl.ds(g * RG, RG)], ksem.at[g])

            def vcp(g):
                return pltpu.make_async_copy(v_hbm.at[pl.ds(g * RG, RG), pl.ds(Z, W)],
                                             v_v.at[pl.ds(g * RG, RG)], vsem.at[g])
            for g in range(nG):
                kcp(g).start(); vcp(g).start()

            zbuf[...] = jnp.zeros_like(zbuf)

            c_x.wait(); c_go.wait(); c_wq.wait()
            row = jax.lax.broadcasted_iota(jnp.int32, (8, D), 0)

            def pad8(ref):
                v = ref[...].astype(F32)
                r = jnp.zeros((8, D), F32)
                for b in range(B):
                    r = jnp.where(row == b, jnp.broadcast_to(v[b:b + 1, :], (8, D)), r)
                return r.astype(BF16)
            x8 = pad8(x_v)
            go8 = pad8(go_v)
            CH = 512
            for c in range(HD // CH):
                qc = jnp.dot(x8, wq_v[:, c * CH:(c + 1) * CH], preferred_element_type=F32)
                for j in range(CH // Dh):
                    q_s[c * (CH // Dh) + j] = qc[:, j * Dh:(j + 1) * Dh].astype(BF16).astype(F32)
            c_wo.wait()
            for c in range(HD // CH):
                dc = jax.lax.dot_general(go8, wo_v[c * CH:(c + 1) * CH, :], (((1,), (1,)), ((), ())),
                                         preferred_element_type=F32)
                for j in range(CH // Dh):
                    do_s[c * (CH // Dh) + j] = dc[:, j * Dh:(j + 1) * Dh].astype(BF16).astype(F32)
            acc_out[...] = jnp.zeros_like(acc_out)
            acc_dx[...] = jnp.zeros_like(acc_dx)

            def zero_cp(i, which):
                s = i // nzr
                r = i % nzr
                dst = (dk_hbm, dv_hbm)[which]
                return pltpu.make_async_copy(zbuf, dst.at[pl.ds(s * ZS, ZS), pl.ds(r * ZR, ZR)], wsem.at[0])
            nz_half = nzs * nzr

            def zero_start(i):
                @pl.when(i < nz_half)
                def _():
                    zero_cp(i, 0).start()

                @pl.when(jnp.logical_and(i >= nz_half, i < n_zero))
                def _():
                    zero_cp(i - nz_half, 1).start()

            def zero_wait():
                zero_cp(0, 0).wait()

            for g in range(nG):
                kcp(g).wait()
                if g < nG - LAST_EARLY:
                    vcp(g).wait()
            if do_writes:
                for i in range(DEPTH):
                    zero_cp(i, 0).start()
            for g in range(nG - LAST_EARLY, nG):
                vcp(g).wait()

            def head(h, carry):
                qh = q_s[h]
                doh = do_s[h]
                rows8 = jax.lax.broadcasted_iota(jnp.int32, (8, Dh), 0)
                o8 = jnp.zeros((8, Dh), F32)
                dq8 = jnp.zeros((8, Dh), F32)
                for b in range(B):
                    bh = b * H + h
                    q = qh[b:b + 1, :]
                    do = doh[b:b + 1, :]
                    K = k_v[bh]
                    V = v_v[bh]
                    Qb = jnp.broadcast_to(q, (Dh, Dh)).astype(BF16)
                    DOb = jnp.broadcast_to(do, (Dh, Dh)).astype(BF16)
                    s = jax.lax.dot_general(K, Qb, (((1,), (1,)), ((), ())), preferred_element_type=F32) * scale
                    m = jnp.max(s, axis=0, keepdims=True)
                    e = jnp.exp(s - m)
                    l = jnp.sum(e, axis=0, keepdims=True)
                    rl = 1.0 / l
                    dp = jax.lax.dot_general(V, DOb, (((1,), (1,)), ((), ())), preferred_element_type=F32)
                    delta = jnp.sum(e * dp, axis=0, keepdims=True) * rl
                    o = jnp.sum(e * V.astype(F32), axis=0, keepdims=True) * rl
                    g = e * (dp - delta)
                    dq = jnp.sum(g * K.astype(F32), axis=0, keepdims=True) * (rl * scale)
                    dk_v[bh] = (g * (q * (rl * scale))).astype(BF16)
                    dv_v[bh] = (e * (do * rl)).astype(BF16)
                    o8 = jnp.where(rows8 == b, jnp.broadcast_to(o, (8, Dh)), o8)
                    dq8 = jnp.where(rows8 == b, jnp.broadcast_to(dq, (8, Dh)), dq8)
                o8 = o8.astype(BF16)
                dq8 = dq8.astype(BF16)
                hs = pl.ds(pl.multiple_of(h * Dh, Dh), Dh)
                wo_h = wo_v[hs, :]
                wq_h = wq_v[:, hs]
                acc_out[...] += jnp.dot(o8, wo_h, preferred_element_type=F32)
                acc_dx[...] += jax.lax.dot_general(dq8, wq_h, (((1,), (1,)), ((), ())), preferred_element_type=F32)
                dwq_h = jax.lax.dot_general(x8, dq8, (((0,), (0,)), ((), ())), preferred_element_type=F32)
                dwq_v[:, hs] = dwq_h.astype(BF16)
                dwo_h = jax.lax.dot_general(o8, go8, (((0,), (0,)), ((), ())), preferred_element_type=F32)
                dwo_v[hs, :] = dwo_h.astype(BF16)
                return carry

            def step(h, carry):
                if do_compute:
                    head(h, 0)
                if do_writes:
                    for j in range(PER_STEP):
                        i = DEPTH + h * PER_STEP + j

                        @pl.when(i < n_zero)
                        def _():
                            zero_wait()
                            zero_start(i)
                return carry
            jax.lax.fori_loop(0, H, step, 0)

            out_v[...] = acc_out[0:B, :].astype(BF16)
            dx_v[...] = acc_dx[0:B, :].astype(BF16)
            if do_writes:
                def rest(i, c):
                    zero_wait()
                    zero_start(i)
                    return c
                lo = min(DEPTH + H * PER_STEP, n_zero)
                if lo < n_zero:
                    jax.lax.fori_loop(lo, n_zero, rest, 0)
                c_out = pltpu.make_async_copy(out_v, out_hbm, osem.at[0])
                c_dx = pltpu.make_async_copy(dx_v, dx_hbm, osem.at[1])
                c_out.start(); c_dx.start()

                def data_cp(i, which):
                    s = i // ndr
                    r = i % ndr
                    src = (dk_v, dv_v)[which]
                    dst = (dk_hbm, dv_hbm)[which]
                    return pltpu.make_async_copy(src.at[pl.ds(s * ZS, ZS), pl.ds(r * ZR, ZR)],
                                                 dst.at[pl.ds(s * ZS, ZS), pl.ds(Z + r * ZR, ZR)], wsem.at[0])
                for which in range(2):
                    def dbody(i, c):
                        zero_wait()
                        data_cp(i, which).start()
                        return c
                    jax.lax.fori_loop(0, nzs * ndr, dbody, 0)

                dwq3 = dwq_v.reshape(WQ_S, wq_rows, HD)
                dwo3 = dwo_v.reshape(WO_S, wo_rows, D)

                def wq_cp(i):
                    return pltpu.make_async_copy(dwq3.at[:, pl.ds(i * WQ_R, WQ_R)],
                                                 dwq_hbm.at[:, pl.ds(i * WQ_R, WQ_R)], osem.at[2])

                def wo_cp(i):
                    return pltpu.make_async_copy(dwo3.at[:, pl.ds(i * WO_R, WO_R)],
                                                 dwo_hbm.at[:, pl.ds(i * WO_R, WO_R)], osem.at[3])
                for i in range(n_wq):
                    wq_cp(i).start()
                for i in range(n_wo):
                    wo_cp(i).start()
                for i in range(DEPTH):
                    zero_wait()
                for i in range(n_wq):
                    wq_cp(i).wait()
                for i in range(n_wo):
                    wo_cp(i).wait()
                c_out.wait(); c_dx.wait()

        any_spec = pl.BlockSpec(memory_space=pl.ANY)
        outs = pl.pallas_call(
            kernel,
            out_shape=(
                jax.ShapeDtypeStruct((B, D), BF16),
                jax.ShapeDtypeStruct((B, D), BF16),
                jax.ShapeDtypeStruct((BH, Sk, Dh), BF16),
                jax.ShapeDtypeStruct((BH, Sk, Dh), BF16),
                jax.ShapeDtypeStruct((WQ_S, wq_rows, HD), BF16),
                jax.ShapeDtypeStruct((WO_S, wo_rows, D), BF16),
            ),
            in_specs=[any_spec] * 6,
            out_specs=(any_spec,) * 6,
            scratch_shapes=[
                pltpu.VMEM((B, D), BF16), pltpu.VMEM((B, D), BF16),
                pltpu.VMEM((B, D), BF16), pltpu.VMEM((B, D), BF16),
                pltpu.VMEM((D, HD), BF16), pltpu.VMEM((HD, D), BF16),
                pltpu.VMEM((BH, W, Dh), BF16), pltpu.VMEM((BH, W, Dh), BF16),
                pltpu.VMEM((BH, W, Dh), BF16), pltpu.VMEM((BH, W, Dh), BF16),
                pltpu.VMEM((D, HD), BF16), pltpu.VMEM((HD, D), BF16),
                pltpu.VMEM((ZS, ZR, Dh), BF16),
                pltpu.VMEM((H, 8, Dh), F32), pltpu.VMEM((H, 8, Dh), F32),
                pltpu.VMEM((8, D), F32), pltpu.VMEM((8, D), F32),
                pltpu.SemaphoreType.DMA((4,)),
                pltpu.SemaphoreType.DMA((nG,)), pltpu.SemaphoreType.DMA((nG,)),
                pltpu.SemaphoreType.DMA((1,)), pltpu.SemaphoreType.DMA((4,)),
            ],
            compiler_params=pltpu.CompilerParams(vmem_limit_bytes=110 * 1024 * 1024),
        )(x.reshape(B, D), k_cache.reshape(BH, Sk, Dh), v_cache.reshape(BH, Sk, Dh), wq, wo,
          grad_out.reshape(B, D))
        out, dx, dk, dv, dwq, dwo = outs
        return (out.reshape(B, Sq, D), dx.reshape(B, Sq, D), dk.reshape(k_cache.shape),
                dv.reshape(v_cache.shape), dwq.reshape(wq.shape), dwo.reshape(wo.shape))
    return jax.jit(fn)


_impl = build()


@jax.jit
def pallas_standalone__sliding_block_cached__decode_kernel(x, k_cache, v_cache, wq, wo, grad_out):
    return _impl(x, k_cache, v_cache, wq, wo, grad_out)
```

```python
import functools
import jax
import jax.numpy as jnp
import jax.experimental.pallas as pl
import jax.experimental.pallas.tpu as pltpu

F32 = jnp.float32
BF16 = jnp.bfloat16
NT = (((1,), (1,)), ((), ()))
TN = (((0,), (0,)), ((), ()))


def build(SA=6, NA=3, SB=7, NB=2, ZR=64, PRO=3, do_compute=True,
          WQ_C=1024, WO_S=4, WO_R=8, TAILD=16, semchk=True, boundchk=True, unroll=4,
          RS=8, RA=16, RP=64, dB=10, L=5, lagA=4, E=4, QA=256, OA=128, WOR_S=8, rorder="qokv", allsplit=False,
          wprio=0):

    def fn(x, k_cache, v_cache, wq, wo, grad_out):
        B, Sq, D = x.shape
        _, H, Sk, Dh = k_cache.shape
        W = min(4096, max(256, Sk // 4))
        Z = Sk - W
        BH = B * H
        scale = Dh ** -0.5
        HD = H * Dh
        assert SA * NA + SB * NB == H
        BATCH = W // ZR
        NQ = Sk // W
        NBW = 2 * B
        PER_G = NBW * NQ
        JA = NA * PER_G
        NBAT = (NA + NB) * PER_G
        WQ_S = D // Dh
        wo_rows = HD // WO_S
        hpw = wo_rows // Dh
        wor_rows = HD // WOR_S
        hpr = wor_rows // Dh
        SM = max(SA, SB)
        nP = W // RP

        def kernel(x_hbm, k_hbm, v_hbm, wq_hbm, wo_hbm, go_hbm,
                   out_hbm, dx_hbm, dk_hbm, dv_hbm, dwq_hbm, dwo_hbm,
                   x_v, go_v, out_v, dx_v, wq_v, wo_v, k_v, v_v, dk_v, dv_v, dwq_v, dwo_v,
                   zbuf, acc_out, acc_dx, sem):
            def loop(lo, hi, f, **kw):
                if isinstance(lo, int) and isinstance(hi, int) and hi <= lo:
                    return
                jax.lax.fori_loop(lo, hi, lambda i, c: (f(i), c)[1], 0, **kw)

            wsem = sem.at[2]
            small = [pltpu.make_async_copy(s, d, wsem) for s, d in ((x_hbm, x_v), (go_hbm, go_v))]

            def kv_seg(src, dst):
                def cp(j, w):
                    g = j // nP
                    r = pl.multiple_of((j % nP) * RP + (0, RA)[w], 8)
                    R = (RA, RP - RA)[w]
                    return pltpu.make_async_copy(src.at[pl.ds(g * RS, RS), pl.ds(Z + r, R)],
                                                 dst.at[pl.ds(g * RS, RS), pl.ds(r, R)], sem.at[w])
                return ((BH // RS) * nP, cp)

            def wq_seg():
                ncq = HD // 1024

                def cp(j, w):
                    r = pl.ds(pl.multiple_of((j // ncq) * 8, 8), 8)
                    c = pl.ds(pl.multiple_of((j % ncq) * 1024 + (0, QA)[w], 128), (QA, 1024 - QA)[w])
                    return pltpu.make_async_copy(wq_hbm.at[:, r, c], wq_v.at[:, r, c], sem.at[w])
                return ((Dh // 8) * ncq, cp)

            def wo_seg():
                def cp(j, w):
                    r = pl.ds(pl.multiple_of(j * 8, 8), 8)
                    c = pl.ds(0, OA) if w == 0 else pl.ds(OA, D - OA)
                    return pltpu.make_async_copy(wo_hbm.at[:, r, c], wo_v.at[:, r, c], sem.at[w])
                return (wor_rows // 8, cp)
            segd = dict(q=wq_seg(), o=wo_seg(), k=kv_seg(k_hbm, k_v), v=kv_seg(v_hbm, v_v))
            rsegs = [segd[c] for c in rorder]
            bounds = [0]
            for cnt, _ in rsegs:
                bounds.append(bounds[-1] + cnt)
            N = bounds[-1]

            def seg_of(i):
                for k in range(len(rsegs)):
                    if bounds[k] <= i < bounds[k + 1]:
                        return k
                return None

            def rstep(i0):
                kb, ka, kb2, kw = seg_of(i0), seg_of(i0 + L), seg_of(i0 + dB), seg_of(i0 - lagA)

                def f(i):
                    if kb is not None:
                        rsegs[kb][1](0, 1).wait()
                    if ka is not None:
                        rsegs[ka][1](i + L - bounds[ka], 0).start(priority=0)
                    if kb2 is not None:
                        rsegs[kb2][1](i + dB - bounds[kb2], 1).start(priority=1)
                    if kw is not None:
                        rsegs[kw][1](0, 0).wait()
                return f

            def rrange(lo, hi):
                cuts = sorted({lo, hi} | {b + o for b in bounds for o in (0, -L, -dB, lagA) if lo < b + o < hi})
                for a, b in zip(cuts[:-1], cuts[1:]):
                    loop(a, b, rstep(a))

            for i in range(L):
                rsegs[0][1](i, 0).start(priority=0)
            loop(0, dB, lambda i: rsegs[0][1](i, 1).start(priority=1))
            for c in small:
                c.start()
            zbuf[...] = jnp.zeros_like(zbuf)
            acc_out[...] = jnp.zeros_like(acc_out)
            acc_dx[...] = jnp.zeros_like(acc_dx)
            rrange(0, 8)
            for c in small:
                c.wait()
            rrange(8, N - E)

            dsts = (dk_hbm, dv_hbm)
            srcs = (dk_v, dv_v)

            def zero_cp(which, s0, S, r):
                return pltpu.make_async_copy(zbuf.at[pl.ds(0, S)],
                                             dsts[which].at[pl.ds(s0, S), pl.ds(r * ZR, ZR)], wsem)

            def data_cp(which, s0, S, r):
                return pltpu.make_async_copy(srcs[which].at[pl.ds(s0, S), pl.ds(r * ZR, ZR)],
                                             dsts[which].at[pl.ds(s0, S), pl.ds(Z + r * ZR, ZR)], wsem)

            def wait_s(S):
                zero_cp(0, 0, S, 0).wait()

            loop(0, PRO * BATCH, lambda i: zero_cp(0, 0, SA, i).start(priority=wprio), unroll=unroll)
            rrange(N - E, N + lagA)

            def batch(j, S, head_base, split):
                g = j // PER_G
                r = j % PER_G
                nz = NBW * (NQ - 1)
                bw = jnp.where(split, jnp.where(r < nz, r // (NQ - 1), r - nz), r // NQ)
                qt = jnp.where(split, jnp.where(r < nz, r % (NQ - 1), NQ - 1), r % NQ)
                s0 = (bw // 2) * H + head_base + g * S
                wh = bw % 2
                for which in range(2):
                    @pl.when(jnp.logical_and(wh == which, qt < NQ - 1))
                    def _():
                        loop(0, BATCH, lambda i: (wait_s(S), zero_cp(which, s0, S, qt * BATCH + i).start(priority=wprio)), unroll=unroll)

                    @pl.when(jnp.logical_and(wh == which, qt == NQ - 1))
                    def _():
                        loop(0, BATCH, lambda i: (wait_s(S), data_cp(which, s0, S, i).start(priority=wprio)), unroll=unroll)

            def batch_any(j):
                @pl.when(j < JA)
                def _():
                    batch(j, SA, 0, True if allsplit else j < PER_G)

                @pl.when(jnp.logical_and(j >= JA, j < JA + PRO))
                def _():
                    loop(0, BATCH, lambda i: (wait_s(SA), zero_cp(0, SA * NA, SB, (j - JA) * BATCH + i).start(priority=wprio)), unroll=unroll)

                @pl.when(j >= JA + PRO)
                def _():
                    batch(j - JA, SB, SA * NA, allsplit)

            row = jax.lax.broadcasted_iota(jnp.int32, (8, D), 0)

            def pad8(ref):
                v = ref[...].astype(F32)
                r = jnp.zeros((8, D), F32)
                for b in range(B):
                    r = jnp.where(row == b, jnp.broadcast_to(v[b:b + 1, :], (8, D)), r)
                return r.astype(BF16)
            x8 = pad8(x_v)
            go8 = pad8(go_v)
            rows8 = jax.lax.broadcasted_iota(jnp.int32, (8, Dh), 0)

            def attn(bh, q, do):
                K = k_v[bh]
                V = v_v[bh]
                q8 = jnp.broadcast_to(q, (8, Dh))
                do8 = jnp.broadcast_to(do, (8, Dh))
                s = jax.lax.dot_general(q8.astype(BF16), K, NT, preferred_element_type=F32) * scale
                dp = jax.lax.dot_general(do8.astype(BF16), V, NT, preferred_element_type=F32)
                m = jnp.max(s, axis=1, keepdims=True)
                e = jnp.exp(s - m)
                p = e / jnp.sum(e, axis=1, keepdims=True)
                ds = p * (dp - jnp.sum(p * dp, axis=1, keepdims=True)) * scale
                rw = jax.lax.broadcasted_iota(jnp.int32, (8, W), 0)
                Lm = jnp.where(rw == 0, ds, jnp.where(rw == 1, p, 0.0)).astype(BF16)
                dq = jnp.dot(Lm, K, preferred_element_type=F32)[0:1, :]
                o = jnp.dot(Lm, V, preferred_element_type=F32)[1:2, :]
                R = jnp.concatenate([jnp.where(rows8 == 0, q8, 0.0), jnp.where(rows8 == 1, do8, 0.0)], axis=1).astype(BF16)
                dkv = jax.lax.dot_general(Lm, R, TN, preferred_element_type=F32)
                dk_v[bh] = dkv[:, :Dh].astype(BF16)
                dv_v[bh] = dkv[:, Dh:].astype(BF16)
                return o, dq

            def head(h):
                hs = pl.ds(pl.multiple_of(h * Dh, Dh), Dh)
                wq_h = wq_v[:, :, hs].reshape(D, Dh)
                wo_h = wo_v[h // hpr, pl.ds(pl.multiple_of((h % hpr) * Dh, Dh), Dh), :]
                qh = jnp.dot(x8, wq_h, preferred_element_type=F32).astype(BF16).astype(F32)
                doh = jax.lax.dot_general(go8, wo_h, NT, preferred_element_type=F32).astype(BF16).astype(F32)
                o8 = jnp.zeros((8, Dh), F32)
                dq8 = jnp.zeros((8, Dh), F32)
                for b in range(B):
                    o, dq = attn(b * H + h, qh[b:b + 1, :], doh[b:b + 1, :])
                    o8 = jnp.where(rows8 == b, jnp.broadcast_to(o, (8, Dh)), o8)
                    dq8 = jnp.where(rows8 == b, jnp.broadcast_to(dq, (8, Dh)), dq8)
                o8 = o8.astype(BF16)
                dq8 = dq8.astype(BF16)
                acc_out[...] += jnp.dot(o8, wo_h, preferred_element_type=F32)
                acc_dx[...] += jax.lax.dot_general(dq8, wq_h, NT, preferred_element_type=F32)
                dwq_h = jax.lax.dot_general(x8, dq8, TN, preferred_element_type=F32)
                dwq_v[:, :, hs] = dwq_h.astype(BF16).reshape(WQ_S, Dh, Dh)
                dwo_h = jax.lax.dot_general(o8, go8, TN, preferred_element_type=F32)
                dwo_v[h // hpw, pl.ds(pl.multiple_of((h % hpw) * Dh, Dh), Dh), :] = dwo_h.astype(BF16)

            def cum(t):
                return PRO + 2 * t if allsplit else PRO + t + t // 2
            T = next(t for t in range(H, 10 * H) if cum(t) >= NBAT)

            def tick(t):
                if do_compute:
                    @pl.when(t < H)
                    def _():
                        head(t)
                loop(cum(t), jnp.minimum(cum(t + 1), NBAT), batch_any)
            loop(0, T, tick)

            out_v[...] = acc_out[0:B, :].astype(BF16)
            dx_v[...] = acc_dx[0:B, :].astype(BF16)
            c_out = pltpu.make_async_copy(out_v, out_hbm, sem.at[0])
            c_dx = pltpu.make_async_copy(dx_v, dx_hbm, sem.at[0])
            c_out.start(); c_dx.start()

            ncq = HD // WQ_C

            def wq_cp(i):
                r = pl.ds(pl.multiple_of((i // ncq) * 8, 8), 8)
                c = pl.ds(pl.multiple_of((i % ncq) * WQ_C, 128), WQ_C)
                return pltpu.make_async_copy(dwq_v.at[:, r, c], dwq_hbm.at[:, r, c], wsem)

            def wo_cp(i):
                r = pl.ds(pl.multiple_of(i * WO_R, 8), WO_R)
                return pltpu.make_async_copy(dwo_v.at[:, r], dwo_hbm.at[:, r], wsem)
            tail = [((Dh // 8) * ncq, lambda i: wq_cp(i).start(priority=wprio), lambda: wq_cp(0).wait()),
                    (wo_rows // WO_R, lambda i: wo_cp(i).start(priority=wprio), lambda: wo_cp(0).wait())]
            prev_wait = functools.partial(wait_s, SB)
            loop(0, PRO * BATCH - TAILD, lambda i: prev_wait())
            for cnt, st, wt in tail:
                assert cnt >= TAILD
                loop(0, TAILD, lambda i: (prev_wait(), st(i)))
                loop(TAILD, cnt, lambda i: (wt(), st(i)))
                prev_wait = wt
            c_out.wait(); c_dx.wait()
            loop(0, TAILD, lambda i: prev_wait())

        any_spec = pl.BlockSpec(memory_space=pl.ANY)
        outs = pl.pallas_call(
            kernel,
            out_shape=(
                jax.ShapeDtypeStruct((B, D), BF16),
                jax.ShapeDtypeStruct((B, D), BF16),
                jax.ShapeDtypeStruct((BH, Sk, Dh), BF16),
                jax.ShapeDtypeStruct((BH, Sk, Dh), BF16),
                jax.ShapeDtypeStruct((WQ_S, Dh, HD), BF16),
                jax.ShapeDtypeStruct((WO_S, wo_rows, D), BF16),
            ),
            in_specs=[any_spec] * 6,
            out_specs=(any_spec,) * 6,
            scratch_shapes=[
                pltpu.VMEM((B, D), BF16), pltpu.VMEM((B, D), BF16),
                pltpu.VMEM((B, D), BF16), pltpu.VMEM((B, D), BF16),
                pltpu.VMEM((WQ_S, Dh, HD), BF16), pltpu.VMEM((WOR_S, wor_rows, D), BF16),
                pltpu.VMEM((BH, W, Dh), BF16), pltpu.VMEM((BH, W, Dh), BF16),
                pltpu.VMEM((BH, W, Dh), BF16), pltpu.VMEM((BH, W, Dh), BF16),
                pltpu.VMEM((WQ_S, Dh, HD), BF16), pltpu.VMEM((WO_S, wo_rows, D), BF16),
                pltpu.VMEM((SM, ZR, Dh), BF16),
                pltpu.VMEM((8, D), F32), pltpu.VMEM((8, D), F32),
                pltpu.SemaphoreType.DMA((3,)),
            ],
            compiler_params=pltpu.CompilerParams(vmem_limit_bytes=110 * 1024 * 1024,
                                                 disable_semaphore_checks=not semchk,
                                                 disable_bounds_checks=not boundchk),
        )(x.reshape(B, D), k_cache.reshape(BH, Sk, Dh), v_cache.reshape(BH, Sk, Dh),
          wq.reshape(WQ_S, Dh, HD), wo.reshape(WOR_S, wor_rows, D), grad_out.reshape(B, D))
        out, dx, dk, dv, dwq, dwo = outs
        return (out.reshape(B, Sq, D), dx.reshape(B, Sq, D), dk.reshape(k_cache.shape),
                dv.reshape(v_cache.shape), dwq.reshape(wq.shape), dwo.reshape(wo.shape))
    return jax.jit(fn)


_impl = build()


@jax.jit
def pallas_standalone__sliding_block_cached__decode_kernel(x, k_cache, v_cache, wq, wo, grad_out):
    return _impl(x, k_cache, v_cache, wq, wo, grad_out)
```

```python
import functools

import jax
import jax.numpy as jnp
import jax.experimental.pallas as pl
import jax.experimental.pallas.tpu as pltpu

F32 = jnp.float32
BF16 = jnp.bfloat16
NT = (((1,), (1,)), ((), ()))
TN = (((0,), (0,)), ((), ()))

KV_S = 8
KV_P = 64
KV_A = 16
WQ_P = 1024
WQ_A = 256
WO_RS = 8
WO_A = 128
LEAD_A = 5
LEAD_B = 10
LAG_A = 4
EARLY = 4
GROUPS = ((6, 3), (7, 2))
ZR = 64
PRO = 3
DWQ_C = 1024
DWO_S = 4
DWO_R = 8
TAIL_D = 16


def _loop(lo, hi, body, **kw):
    if isinstance(lo, int) and isinstance(hi, int) and hi <= lo:
        return
    jax.lax.fori_loop(lo, hi, lambda i, c: (body(i), c)[1], 0, **kw)


def _run_all(*thunks):
    for t in thunks:
        t()


@jax.jit
def pallas_standalone__sliding_block_cached__decode_kernel(
    x: jax.Array,
    k_cache: jax.Array,
    v_cache: jax.Array,
    wq: jax.Array,
    wo: jax.Array,
    grad_out: jax.Array,
):
    B, Sq, D = x.shape
    _, H, Sk, Dh = k_cache.shape
    assert Sq == 1 and B <= 8 and wq.shape == (D, H * Dh) and wo.shape == (H * Dh, D)
    W = min(4096, max(256, Sk // 4))
    Z = Sk - W
    BH, HD = B * H, H * Dh
    scale = Dh ** -0.5

    (SA, NA), (SB, NB) = GROUPS
    assert SA * NA + SB * NB == H and Sk % W == 0
    BATCH = W // ZR
    NQ = Sk // W
    NBW = 2 * B
    PER_G = NBW * NQ
    NZ = NBW * (NQ - 1)
    JA = NA * PER_G
    NBAT = (NA + NB) * PER_G
    WQ_S = D // Dh
    wo_rows, dwo_rows = HD // WO_RS, HD // DWO_S
    assert PRO < NQ

    def issued_before(t):
        return PRO + t + t // 2
    n_ticks = next(t for t in range(H, 8 * H) if issued_before(t) >= NBAT)

    for t in range(n_ticks):
        for j in range(issued_before(t), min(issued_before(t + 1), NBAT)):
            g, r = divmod(j, PER_G)
            if (r >= NZ) if g == 0 else (r % NQ == NQ - 1):
                last = (g + 1) * SA if g < NA else NA * SA + (g - NA + 1) * SB
                assert last - 1 <= t, (t, j)

    def kernel(x_hbm, k_hbm, v_hbm, wq_hbm, wo_hbm, go_hbm,
               out_hbm, dx_hbm, dk_hbm, dv_hbm, dwq_hbm, dwo_hbm,
               x_v, go_v, out_v, dx_v, wq_v, wo_v, k_v, v_v, dk_v, dv_v, dwq_v, dwo_v,
               zbuf, acc_out, acc_dx, sem):
        wsem = sem.at[2]

        def kv_seg(src, dst):
            n_p = W // KV_P

            def cp(j, w):
                blocks = pl.ds((j // n_p) * KV_S, KV_S)
                r = pl.multiple_of((j % n_p) * KV_P + (0, KV_A)[w], 8)
                n = (KV_A, KV_P - KV_A)[w]
                return pltpu.make_async_copy(src.at[blocks, pl.ds(Z + r, n)],
                                             dst.at[blocks, pl.ds(r, n)], sem.at[w])
            return (BH // KV_S) * n_p, cp

        def wq_seg():
            n_c = HD // WQ_P

            def cp(j, w):
                r = pl.ds(pl.multiple_of((j // n_c) * 8, 8), 8)
                c = pl.ds(pl.multiple_of((j % n_c) * WQ_P + (0, WQ_A)[w], 128), (WQ_A, WQ_P - WQ_A)[w])
                return pltpu.make_async_copy(wq_hbm.at[:, r, c], wq_v.at[:, r, c], sem.at[w])
            return (Dh // 8) * n_c, cp

        def wo_seg():
            def cp(j, w):
                r = pl.ds(pl.multiple_of(j * 8, 8), 8)
                c = (pl.ds(0, WO_A), pl.ds(WO_A, D - WO_A))[w]
                return pltpu.make_async_copy(wo_hbm.at[:, r, c], wo_v.at[:, r, c], sem.at[w])
            return wo_rows // 8, cp

        segs = [wq_seg(), wo_seg(), kv_seg(k_hbm, k_v), kv_seg(v_hbm, v_v)]
        bounds = [0]
        for cnt, _ in segs:
            bounds.append(bounds[-1] + cnt)
        n_per = bounds[-1]

        def part(i0, w):
            for k, (_, cp) in enumerate(segs):
                if bounds[k] <= i0 < bounds[k + 1]:
                    return lambda i: cp(i - bounds[k], w)
            return None

        def read_steps(lo, hi):
            offs = (0, -LEAD_A, -LEAD_B, LAG_A)
            cuts = sorted({lo, hi} | {b + o for b in bounds for o in offs if lo < b + o < hi})
            for a, b in zip(cuts[:-1], cuts[1:]):
                done_b, next_a = part(a, 1), part(a + LEAD_A, 0)
                next_b, done_a = part(a + LEAD_B, 1), part(a - LAG_A, 0)

                def step(i):
                    if done_b is not None:
                        done_b(a).wait()
                    if next_a is not None:
                        next_a(i + LEAD_A).start(priority=0)
                    if next_b is not None:
                        next_b(i + LEAD_B).start(priority=1)
                    if done_a is not None:
                        done_a(a - LAG_A).wait()
                _loop(a, b, step)

        for i in range(LEAD_A):
            part(0, 0)(i).start(priority=0)
        _loop(0, LEAD_B, lambda i: part(0, 1)(i).start(priority=1))
        small = [pltpu.make_async_copy(x_hbm, x_v, wsem), pltpu.make_async_copy(go_hbm, go_v, wsem)]
        for c in small:
            c.start()
        zbuf[...] = jnp.zeros_like(zbuf)
        acc_out[...] = jnp.zeros_like(acc_out)
        acc_dx[...] = jnp.zeros_like(acc_dx)
        read_steps(0, 2 * LAG_A)
        for c in small:
            c.wait()
        read_steps(2 * LAG_A, n_per - EARLY)

        dsts, srcs = (dk_hbm, dv_hbm), (dk_v, dv_v)

        def zero_cp(which, s0, S, r):
            return pltpu.make_async_copy(zbuf.at[pl.ds(0, S)],
                                         dsts[which].at[pl.ds(s0, S), pl.ds(r * ZR, ZR)], wsem)

        def data_cp(which, s0, S, r):
            return pltpu.make_async_copy(srcs[which].at[pl.ds(s0, S), pl.ds(r * ZR, ZR)],
                                         dsts[which].at[pl.ds(s0, S), pl.ds(Z + r * ZR, ZR)], wsem)

        def wait_kv(S):
            zero_cp(0, 0, S, 0).wait()

        _loop(0, PRO * BATCH, lambda i: zero_cp(0, 0, SA, i).start(), unroll=4)
        read_steps(n_per - EARLY, n_per + LAG_A)

        def paced(S, make):
            _loop(0, BATCH, lambda i: _run_all(functools.partial(wait_kv, S), make(i).start), unroll=4)

        def batch(j, S, head0, zeros_first):
            g, r = j // PER_G, j % PER_G
            pair = jnp.where(zeros_first, jnp.where(r < NZ, r // (NQ - 1), r - NZ), r // NQ)
            slab = jnp.where(zeros_first, jnp.where(r < NZ, r % (NQ - 1), NQ - 1), r % NQ)
            s0 = (pair // 2) * H + head0 + g * S
            for which in range(2):
                @pl.when(jnp.logical_and(pair % 2 == which, slab < NQ - 1))
                def _():
                    paced(S, lambda i: zero_cp(which, s0, S, slab * BATCH + i))

                @pl.when(jnp.logical_and(pair % 2 == which, slab == NQ - 1))
                def _():
                    paced(S, lambda i: data_cp(which, s0, S, i))

        def batch_any(j):
            @pl.when(j < JA)
            def _():
                batch(j, SA, 0, j < PER_G)

            @pl.when(jnp.logical_and(j >= JA, j < JA + PRO))
            def _():
                paced(SA, lambda i: zero_cp(0, SA * NA, SB, (j - JA) * BATCH + i))

            @pl.when(j >= JA + PRO)
            def _():
                batch(j - JA, SB, SA * NA, False)

        def pad8(ref):
            row = jax.lax.broadcasted_iota(jnp.int32, (8, D), 0)
            v = ref[...].astype(F32)
            r = jnp.zeros((8, D), F32)
            for b in range(B):
                r = jnp.where(row == b, jnp.broadcast_to(v[b:b + 1, :], (8, D)), r)
            return r.astype(BF16)
        x8 = pad8(x_v)
        go8 = pad8(go_v)
        row_d = jax.lax.broadcasted_iota(jnp.int32, (8, Dh), 0)

        def attn(bh, q, do):
            K, V = k_v[bh], v_v[bh]
            q8 = jnp.broadcast_to(q, (8, Dh))
            do8 = jnp.broadcast_to(do, (8, Dh))
            s = jax.lax.dot_general(q8.astype(BF16), K, NT, preferred_element_type=F32) * scale
            dp = jax.lax.dot_general(do8.astype(BF16), V, NT, preferred_element_type=F32)
            e = jnp.exp(s - jnp.max(s, axis=1, keepdims=True))
            p = e / jnp.sum(e, axis=1, keepdims=True)
            ds = p * (dp - jnp.sum(p * dp, axis=1, keepdims=True)) * scale
            row_w = jax.lax.broadcasted_iota(jnp.int32, (8, W), 0)
            lhs = jnp.where(row_w == 0, ds, jnp.where(row_w == 1, p, 0.0)).astype(BF16)
            dq = jnp.dot(lhs, K, preferred_element_type=F32)[0:1, :]
            o = jnp.dot(lhs, V, preferred_element_type=F32)[1:2, :]
            rhs = jnp.concatenate([jnp.where(row_d == 0, q8, 0.0), jnp.where(row_d == 1, do8, 0.0)],
                                  axis=1).astype(BF16)
            dkv = jax.lax.dot_general(lhs, rhs, TN, preferred_element_type=F32)
            dk_v[bh] = dkv[:, :Dh].astype(BF16)
            dv_v[bh] = dkv[:, Dh:].astype(BF16)
            return o, dq

        def head_rows(h, rows):
            per = rows // Dh
            return h // per, pl.ds(pl.multiple_of((h % per) * Dh, Dh), Dh)

        def head(h):
            cols = pl.ds(pl.multiple_of(h * Dh, Dh), Dh)
            wq_h = wq_v[:, :, cols].reshape(D, Dh)
            st, rows = head_rows(h, wo_rows)
            wo_h = wo_v[st, rows, :]
            qh = jnp.dot(x8, wq_h, preferred_element_type=F32).astype(BF16).astype(F32)
            doh = jax.lax.dot_general(go8, wo_h, NT, preferred_element_type=F32).astype(BF16).astype(F32)
            o8 = jnp.zeros((8, Dh), F32)
            dq8 = jnp.zeros((8, Dh), F32)
            for b in range(B):
                o, dq = attn(b * H + h, qh[b:b + 1, :], doh[b:b + 1, :])
                o8 = jnp.where(row_d == b, jnp.broadcast_to(o, (8, Dh)), o8)
                dq8 = jnp.where(row_d == b, jnp.broadcast_to(dq, (8, Dh)), dq8)
            o8, dq8 = o8.astype(BF16), dq8.astype(BF16)
            acc_out[...] += jnp.dot(o8, wo_h, preferred_element_type=F32)
            acc_dx[...] += jax.lax.dot_general(dq8, wq_h, NT, preferred_element_type=F32)
            dwq_h = jax.lax.dot_general(x8, dq8, TN, preferred_element_type=F32)
            dwq_v[:, :, cols] = dwq_h.astype(BF16).reshape(WQ_S, Dh, Dh)
            st, rows = head_rows(h, dwo_rows)
            dwo_v[st, rows, :] = jax.lax.dot_general(o8, go8, TN, preferred_element_type=F32).astype(BF16)

        def tick(t):
            @pl.when(t < H)
            def _():
                head(t)
            _loop(issued_before(t), jnp.minimum(issued_before(t + 1), NBAT), batch_any)
        _loop(0, n_ticks, tick)

        out_v[...] = acc_out[0:B, :].astype(BF16)
        dx_v[...] = acc_dx[0:B, :].astype(BF16)
        small = [pltpu.make_async_copy(out_v, out_hbm, sem.at[0]), pltpu.make_async_copy(dx_v, dx_hbm, sem.at[0])]
        for c in small:
            c.start()

        def dwq_cp(i):
            n_c = HD // DWQ_C
            r = pl.ds(pl.multiple_of((i // n_c) * 8, 8), 8)
            c = pl.ds(pl.multiple_of((i % n_c) * DWQ_C, 128), DWQ_C)
            return pltpu.make_async_copy(dwq_v.at[:, r, c], dwq_hbm.at[:, r, c], wsem)

        def dwo_cp(i):
            r = pl.ds(pl.multiple_of(i * DWO_R, 8), DWO_R)
            return pltpu.make_async_copy(dwo_v.at[:, r], dwo_hbm.at[:, r], wsem)

        retire = functools.partial(wait_kv, SB)
        _loop(0, PRO * BATCH - TAIL_D, lambda i: retire())
        for cnt, cp in (((Dh // 8) * (HD // DWQ_C), dwq_cp), (dwo_rows // DWO_R, dwo_cp)):
            _loop(0, TAIL_D, lambda i: _run_all(retire, cp(i).start))
            retire = lambda cp=cp: cp(0).wait()
            _loop(TAIL_D, cnt, lambda i: _run_all(retire, cp(i).start))
        for c in small:
            c.wait()
        _loop(0, TAIL_D, lambda i: retire())

    hbm = pl.BlockSpec(memory_space=pl.ANY)
    vmem = lambda *shape, dtype=BF16: pltpu.VMEM(shape, dtype)
    out, dx, dk, dv, dwq, dwo = pl.pallas_call(
        kernel,
        out_shape=(
            jax.ShapeDtypeStruct((B, D), BF16),
            jax.ShapeDtypeStruct((B, D), BF16),
            jax.ShapeDtypeStruct((BH, Sk, Dh), BF16),
            jax.ShapeDtypeStruct((BH, Sk, Dh), BF16),
            jax.ShapeDtypeStruct((WQ_S, Dh, HD), BF16),
            jax.ShapeDtypeStruct((DWO_S, dwo_rows, D), BF16),
        ),
        in_specs=[hbm] * 6,
        out_specs=(hbm,) * 6,
        scratch_shapes=[
            vmem(B, D), vmem(B, D), vmem(B, D), vmem(B, D),
            vmem(WQ_S, Dh, HD), vmem(WO_RS, wo_rows, D),
            vmem(BH, W, Dh), vmem(BH, W, Dh),
            vmem(BH, W, Dh), vmem(BH, W, Dh),
            vmem(WQ_S, Dh, HD), vmem(DWO_S, dwo_rows, D),
            vmem(max(SA, SB), ZR, Dh),
            vmem(8, D, dtype=F32), vmem(8, D, dtype=F32),
            pltpu.SemaphoreType.DMA((3,)),
        ],
        compiler_params=pltpu.CompilerParams(vmem_limit_bytes=110 * 1024 * 1024),
    )(x.reshape(B, D), k_cache.reshape(BH, Sk, Dh), v_cache.reshape(BH, Sk, Dh),
      wq.reshape(WQ_S, Dh, HD), wo.reshape(WO_RS, wo_rows, D), grad_out.reshape(B, D))
    return (out.reshape(B, Sq, D), dx.reshape(B, Sq, D), dk.reshape(k_cache.shape),
            dv.reshape(v_cache.shape), dwq.reshape(wq.shape), dwo.reshape(wo.shape))
```

```python
import functools

import jax
import jax.numpy as jnp
import jax.experimental.pallas as pl
import jax.experimental.pallas.tpu as pltpu

F32 = jnp.float32
BF16 = jnp.bfloat16
NT = (((1,), (1,)), ((), ()))
TN = (((0,), (0,)), ((), ()))

KV_S = 8
KV_P = 64
KV_A = 16
WQ_P = 1024
WQ_A = 256
WO_RS = 8
WO_A = 128
LEAD_A = 5
LEAD_B = 10
LAG_A = 4
EARLY = 4
GROUPS = ((6, 3), (7, 2))
ZR = 64
PRO = 3
DWQ_C = 1024
DWO_S = 4
DWO_R = 8
TAIL_D = 16


def _loop(lo, hi, body, **kw):
    if isinstance(lo, int) and isinstance(hi, int) and hi <= lo:
        return
    jax.lax.fori_loop(lo, hi, lambda i, c: (body(i), c)[1], 0, **kw)


def _run_all(*thunks):
    for t in thunks:
        t()


@jax.jit
def pallas_standalone__sliding_block_cached__decode_kernel(
    x: jax.Array,
    k_cache: jax.Array,
    v_cache: jax.Array,
    wq: jax.Array,
    wo: jax.Array,
    grad_out: jax.Array,
):
    B, Sq, D = x.shape
    _, H, Sk, Dh = k_cache.shape
    assert Sq == 1 and B <= 8 and wq.shape == (D, H * Dh) and wo.shape == (H * Dh, D)
    W = min(4096, max(256, Sk // 4))
    Z = Sk - W
    BH, HD = B * H, H * Dh
    scale = Dh ** -0.5

    (SA, NA), (SB, NB) = GROUPS
    assert SA * NA + SB * NB == H and Sk % W == 0
    BATCH = W // ZR
    NQ = Sk // W
    NBW = 2 * B
    PER_G = NBW * NQ
    NZ = NBW * (NQ - 1)
    JA = NA * PER_G
    NBAT = (NA + NB) * PER_G
    WQ_S = D // Dh
    wo_rows, dwo_rows = HD // WO_RS, HD // DWO_S
    assert PRO < NQ

    def issued_before(t):
        return PRO + t + t // 2
    n_ticks = next(t for t in range(H, 8 * H) if issued_before(t) >= NBAT)
    assert H % 2 == 0 and n_ticks >= H + H // 2

    for t in range(n_ticks):
        for j in range(issued_before(t), min(issued_before(t + 1), NBAT)):
            g, r = divmod(j, PER_G)
            if (r >= NZ) if g == 0 else (r % NQ == NQ - 1):
                last = (g + 1) * SA if g < NA else NA * SA + (g - NA + 1) * SB
                assert last - 1 <= t, (t, j)

    def kernel(x_hbm, k_hbm, v_hbm, wq_hbm, wo_hbm, go_hbm,
               out_hbm, dx_hbm, dk_hbm, dv_hbm, dwq_hbm, dwo_hbm,
               x_v, go_v, out_v, dx_v, wq_v, wo_v, k_v, v_v, dk_v, dv_v, dwq_v, dwo_v,
               zbuf, o_s, dq_s, acc_out, acc_dx, sem):
        wsem = sem.at[2]

        def kv_seg(src, dst):
            n_p = W // KV_P

            def cp(j, w):
                blocks = pl.ds((j // n_p) * KV_S, KV_S)
                r = pl.multiple_of((j % n_p) * KV_P + (0, KV_A)[w], 8)
                n = (KV_A, KV_P - KV_A)[w]
                return pltpu.make_async_copy(src.at[blocks, pl.ds(Z + r, n)],
                                             dst.at[blocks, pl.ds(r, n)], sem.at[w])
            return (BH // KV_S) * n_p, cp

        def wq_seg():
            n_c = HD // WQ_P

            def cp(j, w):
                r = pl.ds(pl.multiple_of((j // n_c) * 8, 8), 8)
                c = pl.ds(pl.multiple_of((j % n_c) * WQ_P + (0, WQ_A)[w], 128), (WQ_A, WQ_P - WQ_A)[w])
                return pltpu.make_async_copy(wq_hbm.at[:, r, c], wq_v.at[:, r, c], sem.at[w])
            return (Dh // 8) * n_c, cp

        def wo_seg():
            def cp(j, w):
                r = pl.ds(pl.multiple_of(j * 8, 8), 8)
                c = (pl.ds(0, WO_A), pl.ds(WO_A, D - WO_A))[w]
                return pltpu.make_async_copy(wo_hbm.at[:, r, c], wo_v.at[:, r, c], sem.at[w])
            return wo_rows // 8, cp

        segs = [wq_seg(), wo_seg(), kv_seg(k_hbm, k_v), kv_seg(v_hbm, v_v)]
        bounds = [0]
        for cnt, _ in segs:
            bounds.append(bounds[-1] + cnt)
        n_per = bounds[-1]

        def part(i0, w):
            for k, (_, cp) in enumerate(segs):
                if bounds[k] <= i0 < bounds[k + 1]:
                    return lambda i: cp(i - bounds[k], w)
            return None

        def read_steps(lo, hi):
            offs = (0, -LEAD_A, -LEAD_B, LAG_A)
            cuts = sorted({lo, hi} | {b + o for b in bounds for o in offs if lo < b + o < hi})
            for a, b in zip(cuts[:-1], cuts[1:]):
                done_b, next_a = part(a, 1), part(a + LEAD_A, 0)
                next_b, done_a = part(a + LEAD_B, 1), part(a - LAG_A, 0)

                def step(i):
                    if done_b is not None:
                        done_b(a).wait()
                    if next_a is not None:
                        next_a(i + LEAD_A).start(priority=0)
                    if next_b is not None:
                        next_b(i + LEAD_B).start(priority=1)
                    if done_a is not None:
                        done_a(a - LAG_A).wait()
                _loop(a, b, step)

        for i in range(LEAD_A):
            part(0, 0)(i).start(priority=0)
        _loop(0, LEAD_B, lambda i: part(0, 1)(i).start(priority=1))
        small = [pltpu.make_async_copy(x_hbm, x_v, wsem), pltpu.make_async_copy(go_hbm, go_v, wsem)]
        for c in small:
            c.start()
        zbuf[...] = jnp.zeros_like(zbuf)
        acc_out[...] = jnp.zeros_like(acc_out)
        acc_dx[...] = jnp.zeros_like(acc_dx)
        read_steps(0, 2 * LAG_A)
        for c in small:
            c.wait()
        read_steps(2 * LAG_A, n_per - EARLY)

        dsts, srcs = (dk_hbm, dv_hbm), (dk_v, dv_v)

        def zero_cp(which, s0, S, r):
            return pltpu.make_async_copy(zbuf.at[pl.ds(0, S)],
                                         dsts[which].at[pl.ds(s0, S), pl.ds(r * ZR, ZR)], wsem)

        def data_cp(which, s0, S, r):
            return pltpu.make_async_copy(srcs[which].at[pl.ds(s0, S), pl.ds(r * ZR, ZR)],
                                         dsts[which].at[pl.ds(s0, S), pl.ds(Z + r * ZR, ZR)], wsem)

        def wait_kv(S):
            zero_cp(0, 0, S, 0).wait()

        _loop(0, PRO * BATCH, lambda i: zero_cp(0, 0, SA, i).start(), unroll=4)
        read_steps(n_per - EARLY, n_per + LAG_A)

        def retire_batch(S):
            pltpu.make_async_copy(dk_v.at[pl.ds(0, S)], dk_hbm.at[pl.ds(0, S), pl.ds(0, W)], wsem).wait()

        def paced(S, make):
            retire_batch(S)
            _loop(0, BATCH, lambda i: make(i).start(), unroll=4)

        def batch(j, S, head0, zeros_first):
            g, r = j // PER_G, j % PER_G
            pair = jnp.where(zeros_first, jnp.where(r < NZ, r // (NQ - 1), r - NZ), r // NQ)
            slab = jnp.where(zeros_first, jnp.where(r < NZ, r % (NQ - 1), NQ - 1), r % NQ)
            s0 = (pair // 2) * H + head0 + g * S
            for which in range(2):
                @pl.when(jnp.logical_and(pair % 2 == which, slab < NQ - 1))
                def _():
                    paced(S, lambda i: zero_cp(which, s0, S, slab * BATCH + i))

                @pl.when(jnp.logical_and(pair % 2 == which, slab == NQ - 1))
                def _():
                    paced(S, lambda i: data_cp(which, s0, S, i))

        def batch_any(j):
            @pl.when(j < JA)
            def _():
                batch(j, SA, 0, j < PER_G)

            @pl.when(jnp.logical_and(j >= JA, j < JA + PRO))
            def _():
                paced(SA, lambda i: zero_cp(0, SA * NA, SB, (j - JA) * BATCH + i))

            @pl.when(j >= JA + PRO)
            def _():
                batch(j - JA, SB, SA * NA, False)

        def pad8(ref):
            row = jax.lax.broadcasted_iota(jnp.int32, (8, D), 0)
            v = ref[...].astype(F32)
            r = jnp.zeros((8, D), F32)
            for b in range(B):
                r = jnp.where(row == b, jnp.broadcast_to(v[b:b + 1, :], (8, D)), r)
            return r.astype(BF16)
        x8 = pad8(x_v)
        go8 = pad8(go_v)
        row_d = jax.lax.broadcasted_iota(jnp.int32, (8, Dh), 0)

        def attn(bh, q, do):
            K, V = k_v[bh], v_v[bh]
            q8 = jnp.broadcast_to(q, (8, Dh))
            do8 = jnp.broadcast_to(do, (8, Dh))
            s = jax.lax.dot_general(q8.astype(BF16), K, NT, preferred_element_type=F32) * scale
            dp = jax.lax.dot_general(do8.astype(BF16), V, NT, preferred_element_type=F32)
            e = jnp.exp(s - jnp.max(s, axis=1, keepdims=True))
            p = e / jnp.sum(e, axis=1, keepdims=True)
            ds = p * (dp - jnp.sum(p * dp, axis=1, keepdims=True)) * scale
            row_w = jax.lax.broadcasted_iota(jnp.int32, (8, W), 0)
            lhs = jnp.where(row_w == 0, ds, jnp.where(row_w == 1, p, 0.0)).astype(BF16)
            dq = jnp.dot(lhs, K, preferred_element_type=F32)[0:1, :]
            o = jnp.dot(lhs, V, preferred_element_type=F32)[1:2, :]
            rhs = jnp.concatenate([jnp.where(row_d == 0, q8, 0.0), jnp.where(row_d == 1, do8, 0.0)],
                                  axis=1).astype(BF16)
            dkv = jax.lax.dot_general(lhs, rhs, TN, preferred_element_type=F32)
            dk_v[bh] = dkv[:, :Dh].astype(BF16)
            dv_v[bh] = dkv[:, Dh:].astype(BF16)
            return o, dq

        def head_rows(h, rows):
            per = rows // Dh
            return h // per, pl.ds(pl.multiple_of((h % per) * Dh, Dh), Dh)

        def head_weights(h):
            cols = pl.ds(pl.multiple_of(h * Dh, Dh), Dh)
            st, rows = head_rows(h, wo_rows)
            return cols, wq_v[:, :, cols].reshape(D, Dh), wo_v[st, rows, :]

        def head(h):
            _, wq_h, wo_h = head_weights(h)
            qh = jnp.dot(x8, wq_h, preferred_element_type=F32).astype(BF16).astype(F32)
            doh = jax.lax.dot_general(go8, wo_h, NT, preferred_element_type=F32).astype(BF16).astype(F32)
            o8 = jnp.zeros((8, Dh), F32)
            dq8 = jnp.zeros((8, Dh), F32)
            for b in range(B):
                o, dq = attn(b * H + h, qh[b:b + 1, :], doh[b:b + 1, :])
                o8 = jnp.where(row_d == b, jnp.broadcast_to(o, (8, Dh)), o8)
                dq8 = jnp.where(row_d == b, jnp.broadcast_to(dq, (8, Dh)), dq8)
            o_s[h] = o8
            dq_s[h] = dq8

        def head_proj(h):
            cols, wq_h, wo_h = head_weights(h)
            o8, dq8 = o_s[h].astype(BF16), dq_s[h].astype(BF16)
            acc_out[...] += jnp.dot(o8, wo_h, preferred_element_type=F32)
            acc_dx[...] += jax.lax.dot_general(dq8, wq_h, NT, preferred_element_type=F32)
            dwq_h = jax.lax.dot_general(x8, dq8, TN, preferred_element_type=F32)
            dwq_v[:, :, cols] = dwq_h.astype(BF16).reshape(WQ_S, Dh, Dh)
            st, rows = head_rows(h, dwo_rows)
            dwo_v[st, rows, :] = jax.lax.dot_general(o8, go8, TN, preferred_element_type=F32).astype(BF16)

        def tick(t):
            @pl.when(t < H)
            def _():
                head(t)

            @pl.when(jnp.logical_and(t >= H, t < H + H // 2))
            def _():
                _loop(2 * (t - H), 2 * (t - H) + 2, head_proj)
            _loop(issued_before(t), jnp.minimum(issued_before(t + 1), NBAT), batch_any)
        _loop(0, n_ticks, tick)

        out_v[...] = acc_out[0:B, :].astype(BF16)
        dx_v[...] = acc_dx[0:B, :].astype(BF16)
        small = [pltpu.make_async_copy(out_v, out_hbm, sem.at[0]), pltpu.make_async_copy(dx_v, dx_hbm, sem.at[0])]
        for c in small:
            c.start()

        def dwq_cp(i):
            n_c = HD // DWQ_C
            r = pl.ds(pl.multiple_of((i // n_c) * 8, 8), 8)
            c = pl.ds(pl.multiple_of((i % n_c) * DWQ_C, 128), DWQ_C)
            return pltpu.make_async_copy(dwq_v.at[:, r, c], dwq_hbm.at[:, r, c], wsem)

        def dwo_cp(i):
            r = pl.ds(pl.multiple_of(i * DWO_R, 8), DWO_R)
            return pltpu.make_async_copy(dwo_v.at[:, r], dwo_hbm.at[:, r], wsem)

        retire = functools.partial(wait_kv, SB)
        _loop(0, PRO * BATCH - TAIL_D, lambda i: retire())
        for cnt, cp in (((Dh // 8) * (HD // DWQ_C), dwq_cp), (dwo_rows // DWO_R, dwo_cp)):
            _loop(0, TAIL_D, lambda i: _run_all(retire, cp(i).start))
            retire = lambda cp=cp: cp(0).wait()
            _loop(TAIL_D, cnt, lambda i: _run_all(retire, cp(i).start))
        for c in small:
            c.wait()
        _loop(0, TAIL_D, lambda i: retire())

    hbm = pl.BlockSpec(memory_space=pl.ANY)
    vmem = lambda *shape, dtype=BF16: pltpu.VMEM(shape, dtype)
    out, dx, dk, dv, dwq, dwo = pl.pallas_call(
        kernel,
        out_shape=(
            jax.ShapeDtypeStruct((B, D), BF16),
            jax.ShapeDtypeStruct((B, D), BF16),
            jax.ShapeDtypeStruct((BH, Sk, Dh), BF16),
            jax.ShapeDtypeStruct((BH, Sk, Dh), BF16),
            jax.ShapeDtypeStruct((WQ_S, Dh, HD), BF16),
            jax.ShapeDtypeStruct((DWO_S, dwo_rows, D), BF16),
        ),
        in_specs=[hbm] * 6,
        out_specs=(hbm,) * 6,
        scratch_shapes=[
            vmem(B, D), vmem(B, D), vmem(B, D), vmem(B, D),
            vmem(WQ_S, Dh, HD), vmem(WO_RS, wo_rows, D),
            vmem(BH, W, Dh), vmem(BH, W, Dh),
            vmem(BH, W, Dh), vmem(BH, W, Dh),
            vmem(WQ_S, Dh, HD), vmem(DWO_S, dwo_rows, D),
            vmem(max(SA, SB), ZR, Dh),
            vmem(H, 8, Dh, dtype=F32), vmem(H, 8, Dh, dtype=F32),
            vmem(8, D, dtype=F32), vmem(8, D, dtype=F32),
            pltpu.SemaphoreType.DMA((3,)),
        ],
        compiler_params=pltpu.CompilerParams(vmem_limit_bytes=110 * 1024 * 1024),
    )(x.reshape(B, D), k_cache.reshape(BH, Sk, Dh), v_cache.reshape(BH, Sk, Dh),
      wq.reshape(WQ_S, Dh, HD), wo.reshape(WO_RS, wo_rows, D), grad_out.reshape(B, D))
    return (out.reshape(B, Sq, D), dx.reshape(B, Sq, D), dk.reshape(k_cache.shape),
            dv.reshape(v_cache.shape), dwq.reshape(wq.shape), dwo.reshape(wo.shape))
```

```python
import functools

import jax
import jax.numpy as jnp
import jax.experimental.pallas as pl
import jax.experimental.pallas.tpu as pltpu

F32 = jnp.float32
BF16 = jnp.bfloat16
NT = (((1,), (1,)), ((), ()))
TN = (((0,), (0,)), ((), ()))

KV_GROUPS = ((6, 3), (8, 5), (6, 1))
KV_P = 64
KV_A = 16
WQ_P = 1024
WQ_A = 256
WO_RS = 8
WO_A = 128
LEAD_A = 5
LEAD_B = 10
LAG_A = 4
EARLY = 4
GROUPS = ((6, 3), (7, 2))
ZR = 64
PRO = 3
DWQ_C = 1024
DWO_S = 4
DWO_R = 8
TAIL_D = 16


def _loop(lo, hi, body, **kw):
    if isinstance(lo, int) and isinstance(hi, int) and hi <= lo:
        return
    jax.lax.fori_loop(lo, hi, lambda i, c: (body(i), c)[1], 0, **kw)


def _run_all(*thunks):
    for t in thunks:
        t()


@jax.jit
def pallas_standalone__sliding_block_cached__decode_kernel(
    x: jax.Array,
    k_cache: jax.Array,
    v_cache: jax.Array,
    wq: jax.Array,
    wo: jax.Array,
    grad_out: jax.Array,
):
    B, Sq, D = x.shape
    _, H, Sk, Dh = k_cache.shape
    assert Sq == 1 and B <= 8 and wq.shape == (D, H * Dh) and wo.shape == (H * Dh, D)
    W = min(4096, max(256, Sk // 4))
    Z = Sk - W
    BH, HD = B * H, H * Dh
    scale = Dh ** -0.5

    (SA, NA), (SB, NB) = GROUPS
    assert SA * NA + SB * NB == H and Sk % W == 0 and sum(s * n for s, n in KV_GROUPS) == BH
    BATCH = W // ZR
    NQ = Sk // W
    NBW = 2 * B
    PER_G = NBW * NQ
    NZ = NBW * (NQ - 1)
    JA = NA * PER_G
    NBAT = (NA + NB) * PER_G
    WQ_S = D // Dh
    wo_rows, dwo_rows = HD // WO_RS, HD // DWO_S
    assert PRO < NQ

    def issued_before(t):
        return PRO + t + t // 2
    n_ticks = next(t for t in range(H, 8 * H) if issued_before(t) >= NBAT)
    assert H % 2 == 0 and n_ticks >= H + H // 2

    for t in range(n_ticks):
        for j in range(issued_before(t), min(issued_before(t + 1), NBAT)):
            g, r = divmod(j, PER_G)
            if (r >= NZ) if g == 0 else (r % NQ == NQ - 1):
                last = (g + 1) * SA if g < NA else NA * SA + (g - NA + 1) * SB
                assert last - 1 <= t, (t, j)

    def kernel(x_hbm, k_hbm, v_hbm, wq_hbm, wo_hbm, go_hbm,
               out_hbm, dx_hbm, dk_hbm, dv_hbm, dwq_hbm, dwo_hbm,
               x_v, go_v, out_v, dx_v, wq_v, wo_v, k_v, v_v, dk_v, dv_v, dwq_v, dwo_v,
               zbuf, o_s, dq_s, acc_out, acc_dx, sem):
        wsem = sem.at[2]

        def kv_seg(src, dst, first, S, count):
            n_p = W // KV_P

            def cp(j, w):
                blocks = pl.ds(first + (j // n_p) * S, S)
                r = pl.multiple_of((j % n_p) * KV_P + (0, KV_A)[w], 8)
                n = (KV_A, KV_P - KV_A)[w]
                return pltpu.make_async_copy(src.at[blocks, pl.ds(Z + r, n)],
                                             dst.at[blocks, pl.ds(r, n)], sem.at[w])
            return count * n_p, cp

        def wq_seg():
            n_c = HD // WQ_P

            def cp(j, w):
                r = pl.ds(pl.multiple_of((j // n_c) * 8, 8), 8)
                c = pl.ds(pl.multiple_of((j % n_c) * WQ_P + (0, WQ_A)[w], 128), (WQ_A, WQ_P - WQ_A)[w])
                return pltpu.make_async_copy(wq_hbm.at[:, r, c], wq_v.at[:, r, c], sem.at[w])
            return (Dh // 8) * n_c, cp

        def wo_seg():
            def cp(j, w):
                r = pl.ds(pl.multiple_of(j * 8, 8), 8)
                c = (pl.ds(0, WO_A), pl.ds(WO_A, D - WO_A))[w]
                return pltpu.make_async_copy(wo_hbm.at[:, r, c], wo_v.at[:, r, c], sem.at[w])
            return wo_rows // 8, cp

        segs = [wq_seg(), wo_seg()]
        for src, dst in ((k_hbm, k_v), (v_hbm, v_v)):
            first = 0
            for S, count in KV_GROUPS:
                segs.append(kv_seg(src, dst, first, S, count))
                first += S * count
        bounds = [0]
        for cnt, _ in segs:
            bounds.append(bounds[-1] + cnt)
        n_per = bounds[-1]

        def part(i0, w):
            for k, (_, cp) in enumerate(segs):
                if bounds[k] <= i0 < bounds[k + 1]:
                    return lambda i: cp(i - bounds[k], w)
            return None

        def read_steps(lo, hi):
            offs = (0, -LEAD_A, -LEAD_B, LAG_A)
            cuts = sorted({lo, hi} | {b + o for b in bounds for o in offs if lo < b + o < hi})
            for a, b in zip(cuts[:-1], cuts[1:]):
                done_b, next_a = part(a, 1), part(a + LEAD_A, 0)
                next_b, done_a = part(a + LEAD_B, 1), part(a - LAG_A, 0)

                def step(i):
                    if done_b is not None:
                        done_b(a).wait()
                    if next_a is not None:
                        next_a(i + LEAD_A).start(priority=0)
                    if next_b is not None:
                        next_b(i + LEAD_B).start(priority=1)
                    if done_a is not None:
                        done_a(a - LAG_A).wait()
                _loop(a, b, step)

        for i in range(LEAD_A):
            part(0, 0)(i).start(priority=0)
        _loop(0, LEAD_B, lambda i: part(0, 1)(i).start(priority=1))
        small = [pltpu.make_async_copy(x_hbm, x_v, wsem), pltpu.make_async_copy(go_hbm, go_v, wsem)]
        for c in small:
            c.start()
        zbuf[...] = jnp.zeros_like(zbuf)
        acc_out[...] = jnp.zeros_like(acc_out)
        acc_dx[...] = jnp.zeros_like(acc_dx)
        read_steps(0, 2 * LAG_A)
        for c in small:
            c.wait()
        read_steps(2 * LAG_A, n_per - EARLY)

        dsts, srcs = (dk_hbm, dv_hbm), (dk_v, dv_v)

        def zero_cp(which, s0, S, r):
            return pltpu.make_async_copy(zbuf.at[pl.ds(0, S)],
                                         dsts[which].at[pl.ds(s0, S), pl.ds(r * ZR, ZR)], wsem)

        def data_cp(which, s0, S, r):
            return pltpu.make_async_copy(srcs[which].at[pl.ds(s0, S), pl.ds(r * ZR, ZR)],
                                         dsts[which].at[pl.ds(s0, S), pl.ds(Z + r * ZR, ZR)], wsem)

        def wait_kv(S):
            zero_cp(0, 0, S, 0).wait()

        _loop(0, PRO * BATCH, lambda i: zero_cp(0, 0, SA, i).start(), unroll=4)
        read_steps(n_per - EARLY, n_per + LAG_A)

        def retire_batch(S):
            pltpu.make_async_copy(dk_v.at[pl.ds(0, S)], dk_hbm.at[pl.ds(0, S), pl.ds(0, W)], wsem).wait()

        def paced(S, make):
            retire_batch(S)
            _loop(0, BATCH, lambda i: make(i).start(), unroll=4)

        def batch(j, S, head0, zeros_first):
            g, r = j // PER_G, j % PER_G
            pair = jnp.where(zeros_first, jnp.where(r < NZ, r // (NQ - 1), r - NZ), r // NQ)
            slab = jnp.where(zeros_first, jnp.where(r < NZ, r % (NQ - 1), NQ - 1), r % NQ)
            s0 = (pair // 2) * H + head0 + g * S
            for which in range(2):
                @pl.when(jnp.logical_and(pair % 2 == which, slab < NQ - 1))
                def _():
                    paced(S, lambda i: zero_cp(which, s0, S, slab * BATCH + i))

                @pl.when(jnp.logical_and(pair % 2 == which, slab == NQ - 1))
                def _():
                    paced(S, lambda i: data_cp(which, s0, S, i))

        def batch_any(j):
            @pl.when(j < JA)
            def _():
                batch(j, SA, 0, j < PER_G)

            @pl.when(jnp.logical_and(j >= JA, j < JA + PRO))
            def _():
                paced(SA, lambda i: zero_cp(0, SA * NA, SB, (j - JA) * BATCH + i))

            @pl.when(j >= JA + PRO)
            def _():
                batch(j - JA, SB, SA * NA, False)

        def pad8(ref):
            row = jax.lax.broadcasted_iota(jnp.int32, (8, D), 0)
            v = ref[...].astype(F32)
            r = jnp.zeros((8, D), F32)
            for b in range(B):
                r = jnp.where(row == b, jnp.broadcast_to(v[b:b + 1, :], (8, D)), r)
            return r.astype(BF16)
        x8 = pad8(x_v)
        go8 = pad8(go_v)
        row_d = jax.lax.broadcasted_iota(jnp.int32, (8, Dh), 0)

        def attn(bh, q, do):
            K, V = k_v[bh], v_v[bh]
            q8 = jnp.broadcast_to(q, (8, Dh))
            do8 = jnp.broadcast_to(do, (8, Dh))
            s = jax.lax.dot_general(q8.astype(BF16), K, NT, preferred_element_type=F32) * scale
            dp = jax.lax.dot_general(do8.astype(BF16), V, NT, preferred_element_type=F32)
            e = jnp.exp(s - jnp.max(s, axis=1, keepdims=True))
            p = e / jnp.sum(e, axis=1, keepdims=True)
            ds = p * (dp - jnp.sum(p * dp, axis=1, keepdims=True)) * scale
            row_w = jax.lax.broadcasted_iota(jnp.int32, (8, W), 0)
            lhs = jnp.where(row_w == 0, ds, jnp.where(row_w == 1, p, 0.0)).astype(BF16)
            dq = jnp.dot(lhs, K, preferred_element_type=F32)[0:1, :]
            o = jnp.dot(lhs, V, preferred_element_type=F32)[1:2, :]
            rhs = jnp.concatenate([jnp.where(row_d == 0, q8, 0.0), jnp.where(row_d == 1, do8, 0.0)],
                                  axis=1).astype(BF16)
            dkv = jax.lax.dot_general(lhs, rhs, TN, preferred_element_type=F32)
            dk_v[bh] = dkv[:, :Dh].astype(BF16)
            dv_v[bh] = dkv[:, Dh:].astype(BF16)
            return o, dq

        def head_rows(h, rows):
            per = rows // Dh
            return h // per, pl.ds(pl.multiple_of((h % per) * Dh, Dh), Dh)

        def head_weights(h):
            cols = pl.ds(pl.multiple_of(h * Dh, Dh), Dh)
            st, rows = head_rows(h, wo_rows)
            return cols, wq_v[:, :, cols].reshape(D, Dh), wo_v[st, rows, :]

        def head(h):
            _, wq_h, wo_h = head_weights(h)
            qh = jnp.dot(x8, wq_h, preferred_element_type=F32).astype(BF16).astype(F32)
            doh = jax.lax.dot_general(go8, wo_h, NT, preferred_element_type=F32).astype(BF16).astype(F32)
            o8 = jnp.zeros((8, Dh), F32)
            dq8 = jnp.zeros((8, Dh), F32)
            for b in range(B):
                o, dq = attn(b * H + h, qh[b:b + 1, :], doh[b:b + 1, :])
                o8 = jnp.where(row_d == b, jnp.broadcast_to(o, (8, Dh)), o8)
                dq8 = jnp.where(row_d == b, jnp.broadcast_to(dq, (8, Dh)), dq8)
            o_s[h] = o8
            dq_s[h] = dq8

        def head_proj(h):
            cols, wq_h, wo_h = head_weights(h)
            o8, dq8 = o_s[h].astype(BF16), dq_s[h].astype(BF16)
            acc_out[...] += jnp.dot(o8, wo_h, preferred_element_type=F32)
            acc_dx[...] += jax.lax.dot_general(dq8, wq_h, NT, preferred_element_type=F32)
            dwq_h = jax.lax.dot_general(x8, dq8, TN, preferred_element_type=F32)
            dwq_v[:, :, cols] = dwq_h.astype(BF16).reshape(WQ_S, Dh, Dh)
            st, rows = head_rows(h, dwo_rows)
            dwo_v[st, rows, :] = jax.lax.dot_general(o8, go8, TN, preferred_element_type=F32).astype(BF16)

        def tick(t):
            @pl.when(t < H)
            def _():
                head(t)

            @pl.when(jnp.logical_and(t >= H, t < H + H // 2))
            def _():
                _loop(2 * (t - H), 2 * (t - H) + 2, head_proj)
            _loop(issued_before(t), jnp.minimum(issued_before(t + 1), NBAT), batch_any)
        _loop(0, n_ticks, tick)

        out_v[...] = acc_out[0:B, :].astype(BF16)
        dx_v[...] = acc_dx[0:B, :].astype(BF16)
        small = [pltpu.make_async_copy(out_v, out_hbm, sem.at[0]), pltpu.make_async_copy(dx_v, dx_hbm, sem.at[0])]
        for c in small:
            c.start()

        def dwq_cp(i):
            n_c = HD // DWQ_C
            r = pl.ds(pl.multiple_of((i // n_c) * 8, 8), 8)
            c = pl.ds(pl.multiple_of((i % n_c) * DWQ_C, 128), DWQ_C)
            return pltpu.make_async_copy(dwq_v.at[:, r, c], dwq_hbm.at[:, r, c], wsem)

        def dwo_cp(i):
            r = pl.ds(pl.multiple_of(i * DWO_R, 8), DWO_R)
            return pltpu.make_async_copy(dwo_v.at[:, r], dwo_hbm.at[:, r], wsem)

        retire = functools.partial(wait_kv, SB)
        _loop(0, PRO * BATCH - TAIL_D, lambda i: retire())
        for cnt, cp in (((Dh // 8) * (HD // DWQ_C), dwq_cp), (dwo_rows // DWO_R, dwo_cp)):
            _loop(0, TAIL_D, lambda i: _run_all(retire, cp(i).start))
            retire = lambda cp=cp: cp(0).wait()
            _loop(TAIL_D, cnt, lambda i: _run_all(retire, cp(i).start))
        for c in small:
            c.wait()
        _loop(0, TAIL_D, lambda i: retire())

    hbm = pl.BlockSpec(memory_space=pl.ANY)
    vmem = lambda *shape, dtype=BF16: pltpu.VMEM(shape, dtype)
    out, dx, dk, dv, dwq, dwo = pl.pallas_call(
        kernel,
        out_shape=(
            jax.ShapeDtypeStruct((B, D), BF16),
            jax.ShapeDtypeStruct((B, D), BF16),
            jax.ShapeDtypeStruct((BH, Sk, Dh), BF16),
            jax.ShapeDtypeStruct((BH, Sk, Dh), BF16),
            jax.ShapeDtypeStruct((WQ_S, Dh, HD), BF16),
            jax.ShapeDtypeStruct((DWO_S, dwo_rows, D), BF16),
        ),
        in_specs=[hbm] * 6,
        out_specs=(hbm,) * 6,
        scratch_shapes=[
            vmem(B, D), vmem(B, D), vmem(B, D), vmem(B, D),
            vmem(WQ_S, Dh, HD), vmem(WO_RS, wo_rows, D),
            vmem(BH, W, Dh), vmem(BH, W, Dh),
            vmem(BH, W, Dh), vmem(BH, W, Dh),
            vmem(WQ_S, Dh, HD), vmem(DWO_S, dwo_rows, D),
            vmem(max(SA, SB), ZR, Dh),
            vmem(H, 8, Dh, dtype=F32), vmem(H, 8, Dh, dtype=F32),
            vmem(8, D, dtype=F32), vmem(8, D, dtype=F32),
            pltpu.SemaphoreType.DMA((3,)),
        ],
        compiler_params=pltpu.CompilerParams(vmem_limit_bytes=110 * 1024 * 1024),
    )(x.reshape(B, D), k_cache.reshape(BH, Sk, Dh), v_cache.reshape(BH, Sk, Dh),
      wq.reshape(WQ_S, Dh, HD), wo.reshape(WO_RS, wo_rows, D), grad_out.reshape(B, D))
    return (out.reshape(B, Sq, D), dx.reshape(B, Sq, D), dk.reshape(k_cache.shape),
            dv.reshape(v_cache.shape), dwq.reshape(wq.shape), dwo.reshape(wo.shape))
```
